```python
import jax
import jax.numpy as jnp

def _softmax(x, axis=-1):
    return jax.nn.softmax(x, axis=axis)
def _gelu(x):
    return jax.nn.gelu(x, approximate=True)
def _silu(x):
    return jax.nn.silu(x)
def _sigmoid(x):
    return jax.nn.sigmoid(x)
def _layernorm(x, axis=-1, eps=1e-5):
    m = jnp.mean(x, axis=axis, keepdims=True)
    v = jnp.var(x, axis=axis, keepdims=True)
    return (x - m) / jnp.sqrt(v + eps)
def _scatter_add(tgt, idx, src, axis=0):
    return tgt.at[idx].add(src)
def _segment_sum(src, seg, n):
    return jax.ops.segment_sum(src, seg, n)
class _Rng:
    def __init__(self, key):
        self._k = key
    def _next(self):
        self._k, sub = jax.random.split(self._k)
        return sub
    def normal(self, shape):
        return jax.random.normal(self._next(), shape, dtype=jnp.bfloat16)
    def randint(self, lo, hi, shape):
        return jax.random.randint(self._next(), shape, lo, hi, dtype=jnp.int32)
    def uniform(self, shape, lo=0.0, hi=1.0):
        return jax.random.uniform(self._next(), shape, jnp.bfloat16, lo, hi)
    def permutation(self, n):
        return jax.random.permutation(self._next(), n)


kernel_name = 'concat_heads__sliding_block_cached__compressed_kv_cla__decode'

def setup_inputs():
    _rng = _Rng(jax.random.key(int.from_bytes(__import__("os").urandom(4), "little")))
    _w = (lambda a: (lambda t: t.astype(jnp.bfloat16) if jnp.issubdtype(t.dtype, jnp.floating) else t)(jnp.asarray(a)))
    def _A_setup():
        B, Sq, D = 4, 1, 512
        Hq, Hkv, Sk, Dh = 32, 32, 4096, 128
        assert Hq % Hkv == 0, (Hq, Hkv)
        return {
            "x": _w((lambda *s: _rng.normal(s) * 0.05)(B, Sq, D)),
            "k_cache": _w((lambda *s: _rng.normal(s) * 0.05)(B, Hkv, Sk, Dh)),
            "v_cache": _w((lambda *s: _rng.normal(s) * 0.05)(B, Hkv, Sk, Dh)),
            "wq": _w((lambda *s: _rng.normal(s) * 0.05)(D, Hq * Dh) * (D ** -0.5)),
            "wo": _w((lambda *s: _rng.normal(s) * 0.05)(Hq * Dh, D) * ((Hq * Dh) ** -0.5)),
        }
    _A_in = _A_setup()

    def _B_setup():
        B, H, Sq, Sk, D, M = 4, 32, 1, 4096, 128, 512
        Dc = 4 * D
        return {
            "x": _w((lambda *s: _rng.normal(s) * 0.05)(B, Sq, M)),
            "c_kv": _w((lambda *s: _rng.normal(s) * 0.05)(B, Sk, Dc)),
            "w_q": _w((lambda *s: _rng.normal(s) * 0.05)(M, H, D) * (M ** -0.5)),
            "w_uk": _w((lambda *s: _rng.normal(s) * 0.05)(Dc, H, D) * (Dc ** -0.5)),
            "w_uv": _w((lambda *s: _rng.normal(s) * 0.05)(Dc, H, D) * (Dc ** -0.5)),
            "w_o": _w((lambda *s: _rng.normal(s) * 0.05)(H, D, M) * ((H * D) ** -0.5)),
        }
    _B_in = _B_setup()

    return {
        "A_x": _A_in["x"],
        "A_k_cache": _A_in["k_cache"],
        "A_v_cache": _A_in["v_cache"],
        "A_wq": _A_in["wq"],
        "A_wo": _A_in["wo"],
        "B_x": _B_in["x"],
        "B_c_kv": _B_in["c_kv"],
        "B_w_q": _B_in["w_q"],
        "B_w_uk": _B_in["w_uk"],
        "B_w_uv": _B_in["w_uv"],
        "B_w_o": _B_in["w_o"],
    }

def reference(A_x, A_k_cache, A_v_cache, A_wq, A_wo, B_x, B_c_kv, B_w_q, B_w_uk, B_w_uv, B_w_o):
    def _A_ref(x, k_cache, v_cache, wq, wo):
        B, Sq, D = x.shape
        Hq, Dh = 32, 128
        Hkv, Sk = k_cache.shape[1], k_cache.shape[2]
        W = min(4096, max(256, Sk // 4))
        rep = Hq // Hkv
        q = (lambda x, *d: x.transpose(*d))((x @ wq).reshape(B, Sq, Hq, Dh), 0, 2, 1, 3)
        k = jnp.repeat(k_cache[:, :, Sk - W:, :], rep, axis=1)
        v = jnp.repeat(v_cache[:, :, Sk - W:, :], rep, axis=1)
        scores = jnp.einsum("bhqd,bhkd->bhqk", q, k) * (Dh ** -0.5)
        p = _softmax(scores, axis=-1)
        o = jnp.einsum("bhqk,bhkd->bhqd", p, v)
        return (lambda x, *d: x.transpose(*d))(o, 0, 2, 1, 3).reshape(B, Sq, Hq * Dh) @ wo

    def _B_ref(x, c_kv, w_q, w_uk, w_uv, w_o):
        B, Sq, M = x.shape[0], x.shape[1], x.shape[2]
        Sk = c_kv.shape[1]
        H, D = w_q.shape[1], w_q.shape[2]
        q = jnp.einsum("bqm,mhd->bhqd", x, w_q)
        k = jnp.einsum("bkc,chd->bhkd", c_kv, w_uk)
        v = jnp.einsum("bkc,chd->bhkd", c_kv, w_uv)
        scores = jnp.einsum("bhqd,bhkd->bhqk", q, k) * (D ** -0.5)
        off = Sk - Sq
        qi = jnp.arange(Sq)[:, None]
        kj = jnp.arange(Sk)[None, :]
        cmask = kj <= (qi + off)
        scores = jnp.where(cmask[None, None], scores, -1e9)
        p = _softmax(scores, axis=-1)
        ctx = jnp.einsum("bhqk,bhkd->bhqd", p, v)
        return jnp.einsum("bhqd,hdm->bqm", ctx, w_o)

    a = _A_ref(A_x, A_k_cache, A_v_cache, A_wq, A_wo)
    b = _B_ref(B_x, B_c_kv, B_w_q, B_w_uk, B_w_uv, B_w_o)
    return jnp.concatenate([a, b], axis=-1)
```

```python
import re

import jax
import jax.numpy as jnp
from jax import lax
from jax.experimental import pallas as pl
from jax.experimental.pallas import tpu as pltpu

BF = jnp.bfloat16
F32 = jnp.float32
NT = (((1,), (1,)), ((), ()))
SK, WIN = 4096, 1024


def _dot(a, b):
    return jnp.dot(a, b, preferred_element_type=F32)


def _dot_nt(a, b):
    return lax.dot_general(a, b, NT, preferred_element_type=F32)


def _iota(shape, dim):
    return lax.broadcasted_iota(jnp.int32, shape, dim)


def _loop(n, body, init=None, unroll=False):
    return lax.fori_loop(0, n, body, init, unroll=unroll)


def _al(i, n):
    return pl.ds(i * n if isinstance(i, int) else pl.multiple_of(i * n, n), n)


def make(seg_w="4a4b", seg_c="4a4b", seg_k="4a4b", seg_v="4a4b", seg_o="4a4b", compute="all",
         semchecks=False, tail=4, pw=1, pc=1, pk=1, po=1, flags=None):
    parse = lambda s: [(int(n), "ab".index(c)) for n, c in re.findall(r"(\d+)([ab])", s)]
    NSEM = 4
    on = lambda name: compute == "all" or name in compute

    def kernel(xa_h, k_h, v_h, wq_h, wo_h, xb_h, c_h, bq_h, uk_h, uv_h, bo_h, out_h,
               xa_s, k_s, v_s, wq_s, wo_s, xb_s, c_s, bq_s, uk_s, uv_s, bo_s,
               r_s, x64_s, qb_s, ql_s, sc_s, cl_s, qa_s, lhs_s, out_s, sems, tsems, xsem):
        scale = 128 ** -0.5

        def row(src, dst, seg, sem):
            s0 = 0
            for n, prio in parse(seg):
                pltpu.make_async_copy(src(pl.ds(s0, n)), dst(pl.ds(s0, n)), sem).start(priority=prio)
                s0 += n

        def part(rows, j, n, body):
            per = rows // n
            _loop(per, lambda p, c: body(j * per + p))

        def issue_w3(h, s, sem, j=0, n=1):
            part(64 // pw, j, n, lambda p: row(lambda d: h.at[d, _al(p, pw)], lambda d: s.at[d, _al(p, pw)], seg_w, sem))

        def issue_wq(sem, j=0, n=1):
            def body(p):
                for i in range(8 // pw):
                    col = _al(i, 512 * pw)
                    row(lambda d: wq_h.at[d, _al(p, 8), col], lambda d: wq_s.at[d, _al(p, 8), col], seg_w, sem)
            part(8, j, n, body)

        def issue_rows(h, s, seg, m, sem, j=0, n=1):
            part(64 // m, j, n, lambda p: row(lambda d: h.at[d, _al(p, 8 * m)], lambda d: s.at[d, _al(p, 8 * m)], seg, sem))

        def issue_kv(g, sem, j=0, n=1):
            r = int(32 * pk)
            def body(p):
                src, dst = _al((SK - WIN) // r + p, r), _al(p, r)
                row(lambda d: k_h.at[d, g, src], lambda d: k_s.at[g, d, dst], seg_k, sem)
                row(lambda d: v_h.at[d, g, src], lambda d: v_s.at[g, d, dst], seg_v, sem)
            part(WIN // r, j, n, body)

        def wait(buf, sem):
            pltpu.make_async_copy(buf, buf, sem).wait()

        def sem(i):
            return sems.at[i & (NSEM - 1)]

        def head_mask():
            return (_iota((64, 1024), 0) & 15) == (_iota((64, 1024), 1) & 15)

        def w_blk(w_s, s, t):
            return w_s[s, :, _al(t, 16), :].reshape(1024, 128)

        def expand(x, u):
            return jnp.where(head_mask(), _dot(x, r_s[u]), 0.0).astype(BF)

        def store_lhs(base, g, o):
            top = _iota((8, 128), 0) < 4
            lhs_s[base + g] = jnp.where(top, o, 0.0)
            lhs_s[base + 16 + g] = jnp.where(top, 0.0, o)

        def project(w_s, base, s0, ns, j):
            l = jnp.concatenate([lhs_s[base + 4 * (s0 + s) + j] for s in range(ns)], axis=1).astype(BF)
            w = w_s[pl.ds(s0, ns), _al(j, 128), :].reshape(128 * ns, 512)
            return _dot(l, w)

        def emit(acc, lo):
            out_s[:, lo:lo + 512] = (acc[0:4] + acc[4:8]).astype(BF)

        xcopies = [pltpu.make_async_copy(xa_h, xa_s, xsem), pltpu.make_async_copy(xb_h, xb_s, xsem)]
        for c in xcopies: c.start()
        issue_w3(bq_h, bq_s, sem(0))
        for c in xcopies: c.wait()
        if on("q"):
            def rbody(i, c):
                u, r = i >> 3, i & 7
                hit = (_iota((16, 1024), 0) + 16 * r) == (_iota((16, 1024), 1) >> 4) + 64 * u
                r_s[u, _al(r, 16), :] = jnp.where(hit, 1.0, 0.0).astype(BF)
            _loop(16, rbody)
            xb = xb_s[...].astype(F32)
            for b in range(4):
                for j in range(4):
                    x64_s[j, 16 * b:16 * b + 16, :] = jnp.broadcast_to(
                        xb[b:b + 1, 128 * j:128 * j + 128], (16, 128)).astype(BF)
        issue_w3(uk_h, uk_s, sem(1))

        wait(bq_s, sem(0))
        def qb_step(s, acc):
            issue_wq(sem(2), s, 8)
            if not on("q"): return acc
            xe = expand(x64_s[s >> 1], s & 1)
            return tuple(acc[t] + _dot(xe, w_blk(bq_s, s, t)) for t in range(2))
        q = _loop(8, qb_step, (jnp.zeros((64, 128), F32),) * 2)
        for t in range(2):
            qb_s[t] = q[t].astype(BF)

        wait(uk_s, sem(1))
        def ql_step(i, c):
            issue_rows(c_h.at[0], c_s.at[0], seg_c, pc, sem(3), i, 8)
            if not on("l"): return
            j, t = i >> 1, i & 1
            def half(u, res):
                full = _dot_nt(qb_s[t], w_blk(uk_s, 2 * j + u, t))
                sel = jnp.where(head_mask(), full, 0.0).astype(BF)
                return res + _dot_nt(sel, r_s[u])
            res = _loop(2, half, jnp.zeros((64, 128), F32)).astype(BF)
            for b in range(4):
                ql_s[b, j, _al(t, 16), :] = res[16 * b:16 * b + 16]
        _loop(8, ql_step)

        wait(wq_s, sem(2))
        xa = xa_s[...].astype(F32)
        x8 = jnp.concatenate([xa, xa], axis=0).astype(BF)
        def qa_step(i, c):
            issue_rows(c_h.at[1], c_s.at[1], seg_c, pc, sem(4), i, 8)
            if not on("a"): return
            q = _dot(x8, wq_s[:, :, _al(i, 512)].reshape(512, 512))
            for h in range(4):
                qa_s[4 * i + h] = q[:, 128 * h:128 * h + 128]
        _loop(8, qa_step)

        def c_step(b, c):
            wait(c_s.at[b], sem(3 + b))
            def issue(j):
                nb = jnp.minimum(b + 2, 3)
                pl.when(b < 2)(lambda: issue_rows(c_h.at[nb], c_s.at[nb], seg_c, pc, sem(5 + b), j, 16))
                pl.when(b == 2)(lambda: issue_w3(uv_h, uv_s, sem(7), j, 16))
                pl.when(b == 3)(lambda: issue_rows(bo_h, bo_s, seg_o, po, sem(8), j, 16))
            ql = jnp.concatenate([ql_s[b, j] for j in range(4)], axis=1)

            def body1(j, m):
                issue(j)
                if not on("c"): return m
                s = _dot_nt(ql, c_s[b, j]) * scale
                sc_s[j] = s
                return jnp.maximum(m, s)
            m = _loop(8, body1, jnp.full((32, 512), -jnp.inf, F32))
            m = jnp.max(m, axis=1, keepdims=True)

            def body2(j, carry):
                issue(8 + j)
                if not on("c"): return carry
                l, acc = carry
                p = jnp.exp(sc_s[j] - m)
                return l + p, acc + _dot(p.astype(BF), c_s[b, j])
            l, acc = _loop(8, body2, (jnp.zeros((32, 512), F32),) * 2)
            cl = (acc * (1.0 / jnp.sum(l, axis=1, keepdims=True))).astype(BF)
            for j in range(4):
                for t in range(2):
                    cl_s[j, t, b] = cl[16 * t:16 * t + 16, 128 * j:128 * j + 128]
        _loop(4, c_step)

        wait(uv_s, sem(7))
        def ctx_outer(t, c):
            def ctx_step(s, acc):
                issue_kv(0, sem(9), 8 * t + s, 16)
                if not on("v"): return acc
                return acc + _dot(expand(cl_s[s >> 1, t].reshape(64, 128), s & 1), w_blk(uv_s, s, t))
            qb_s[t] = _loop(8, ctx_step, jnp.zeros((64, 128), F32)).astype(BF)
        _loop(2, ctx_outer)
        r, c = _iota((128, 128), 0), _iota((128, 128), 1)
        perm = jnp.where(c == (r & 7) * 16 + (r >> 3), 1.0, 0.0).astype(BF)
        ctx = _dot(perm, qb_s[...].reshape(128, 128))
        for g in range(16):
            store_lhs(32, g, ctx[8 * g:8 * g + 8])

        wait(bo_s, sem(8))
        def ob_step(i, acc):
            issue_kv(1, sem(10), i, 8)
            if not on("o"): return acc
            return acc + project(bo_s, 32, 4 * (i & 1), 4, i >> 1)
        emit(_loop(8, ob_step, jnp.zeros((8, 512), F32)), 512)

        def kv_step(g, c):
            wait(k_s.at[g], sem(9 + g))
            wait(v_s.at[g], sem(9 + g))
            pl.when(g < 14)(lambda: issue_kv(jnp.minimum(g + 2, 15), sem(11 + g)))
            def issue_wo(j):
                issue_rows(wo_h, wo_s, seg_o, po, tsems.at[j], j, tail)
            pl.when(g >= 14)(lambda: _loop(tail // 2, lambda j, c: issue_wo((g & 1) * (tail // 2) + j)))
            if not on("k"): return
            def qk(i, s):
                si = _dot_nt(qa_s[g + 16 * (i & 1)].astype(BF), k_s[g, i])
                return jnp.where(_iota((8, WIN), 0) == (i & 1) * 4 + (i >> 1), si, s)
            s = _loop(8, qk, jnp.zeros((8, WIN), F32), unroll=2) * scale
            p = jnp.exp(s - jnp.max(s, axis=1, keepdims=True))
            l = jnp.sum(p, axis=1, keepdims=True)
            pb = p.astype(BF)
            def pv(i, o):
                return jnp.where(_iota((8, 128), 0) == (i & 1) * 4 + (i >> 1), _dot(pb, v_s[g, i]), o)
            store_lhs(0, g, _loop(8, pv, jnp.zeros((8, 128), F32), unroll=2) / l)
        _loop(16, kv_step)

        def oa_step(j, acc):
            wait(wo_s.at[:, _al(j, 128)], tsems.at[j])
            if not on("w"): return acc
            return acc + project(wo_s, 0, 0, 8, j)
        emit(_loop(4, oa_step, jnp.zeros((8, 512), F32)), 0)
        oc = pltpu.make_async_copy(out_s, out_h, xsem)
        oc.start()
        oc.wait()

    def f(A_x, A_k_cache, A_v_cache, A_wq, A_wo, B_x, B_c_kv, B_w_q, B_w_uk, B_w_uv, B_w_o):
        vm = pltpu.VMEM
        out = pl.pallas_call(
            kernel,
            out_shape=jax.ShapeDtypeStruct((4, 1024), BF),
            in_specs=[pl.BlockSpec(memory_space=pltpu.HBM)] * 11,
            out_specs=pl.BlockSpec(memory_space=pltpu.HBM),
            scratch_shapes=[
                vm((4, 512), BF), vm((16, 8, WIN, 128), BF), vm((16, 8, WIN, 128), BF),
                vm((8, 64, 4096), BF), vm((8, 512, 512), BF), vm((4, 512), BF), vm((4, 8, 512, 512), BF),
                vm((8, 64, 32, 128), BF), vm((8, 64, 32, 128), BF), vm((8, 64, 32, 128), BF),
                vm((8, 512, 512), BF),
                vm((2, 128, 1024), BF), vm((4, 64, 128), BF), vm((2, 64, 128), BF), vm((4, 4, 32, 128), BF),
                vm((8, 32, 512), F32), vm((4, 2, 4, 16, 128), BF), vm((32, 8, 128), F32),
                vm((64, 8, 128), F32), vm((4, 1024), BF),
                pltpu.SemaphoreType.DMA((NSEM,)), pltpu.SemaphoreType.DMA((tail,)), pltpu.SemaphoreType.DMA,
            ],
            compiler_params=pltpu.CompilerParams(
                vmem_limit_bytes=124 << 20, disable_bounds_checks=True,
                disable_semaphore_checks=not semchecks, flags=flags),
        )(A_x.reshape(4, 512), A_k_cache.reshape(8, 16, SK, 128), A_v_cache.reshape(8, 16, SK, 128),
          A_wq.reshape(8, 64, 4096), A_wo.reshape(8, 512, 512), B_x.reshape(4, 512),
          B_c_kv.reshape(4, 8, 512, 512), B_w_q.reshape(8, 64, 32, 128), B_w_uk.reshape(8, 64, 32, 128),
          B_w_uv.reshape(8, 64, 32, 128), B_w_o.reshape(8, 512, 512))
        return out.reshape(4, 1, 1024)
    return f


_impl = make()


@jax.jit
def pallas_concat_heads__sliding_block_cached__compressed_kv_cla__decode_kernel(
        A_x, A_k_cache, A_v_cache, A_wq, A_wo, B_x, B_c_kv, B_w_q, B_w_uk, B_w_uv, B_w_o):
    return _impl(A_x, A_k_cache, A_v_cache, A_wq, A_wo, B_x, B_c_kv, B_w_q, B_w_uk, B_w_uv, B_w_o)
```

```python
import re
import jax
import jax.numpy as jnp
from jax import lax
from jax.experimental import pallas as pl
from jax.experimental.pallas import tpu as pltpu

BF = jnp.bfloat16
F32 = jnp.float32
NT = (((1,), (1,)), ((), ()))
SK, WIN = 4096, 1024


def _dot(a, b):
    return jnp.dot(a, b, preferred_element_type=F32)


def _dot_nt(a, b):
    return lax.dot_general(a, b, NT, preferred_element_type=F32)


def _iota(shape, dim):
    return lax.broadcasted_iota(jnp.int32, shape, dim)


def _loop(n, body, init=None, unroll=False):
    return lax.fori_loop(0, n, body, init, unroll=unroll)


def _al(i, n):
    return pl.ds(i * n if isinstance(i, int) else pl.multiple_of(i * n, n), n)


def rep(pat, names, mode="sep"):
    pp = [(int(n), c) for n, c in re.findall(r"(\d+)([ab])", pat)]
    tot = sum(n for n, _ in pp)
    out = []
    if mode == "sep":
        for a in names:
            for _ in range((32 if a == "c" else 8) // tot):
                out += [f"{a}{n}{c}" for n, c in pp]
    elif mode == "alt":
        for _ in range(8 // tot):
            for a in names:
                out += [f"{a}{n}{c}" for n, c in pp]
    elif mode == "x":
        m = len(names)
        for _ in range(8 // tot):
            for i in range(m):
                out += [f"{names[(i + k) % m]}{n}{c}" for k, (n, c) in enumerate(pp)]
    return " ".join(out)


def make(p1=("2a6b", "sep", 16), p2=("2a6b", "sep", 16), p3=("2a6b", "sep", 16), p4=("2a6b", "sep", 16),
         hs=16, compute="all", semchecks=False, flags=None, pad=0, pad2=0, stages=(("2a2b", 16), ("1a1b", 32), ("b", 128), ("b", 128)), xfirst=False,
         n1="quwvo", prow=None):
    on = lambda name: compute == "all" or name in compute
    P1, P2, P3, P4 = rep(p1[0], n1, p1[1]), rep(p2[0], "c"), rep(p3[0], "KV", p3[1]), rep(p4[0], "a", p4[1])
    GO = 16 // hs

    def kernel(xa_h, k_h, v_h, wq_h, wo_h, xb_h, c_h, bq_h, uk_h, uv_h, bo_h, out_h,
               xa_s, k_s, v_s, wq_s, wo_s, xb_s, c_s, bq_s, uk_s, uv_s, bo_s,
               r_s, x64_s, qb_s, ql_s, sc_s, cl_s, qa_s, oa_s, ob_s, out_s, sems, xsem):
        scale = 128 ** -0.5

        def views(a, d, p, ck, g):
            if a in "quv":
                h, s = dict(q=(bq_h, bq_s), u=(uk_h, uk_s), v=(uv_h, uv_s))[a]
                return h.at[d, _al(p, ck // 8)], s.at[d, _al(p, ck // 8)]
            if a == "w":
                m = 64 // ck
                ix = (d, _al(p // m, 8), _al(p & (m - 1), 64 * ck))
                return wq_h.at[ix], wq_s.at[ix]
            if a in "coa":
                h, s = dict(c=(c_h, c_s), o=(bo_h, bo_s), a=(wo_h, wo_s))[a]
                return h.at[d, _al(p, ck)], s.at[d, _al(p, ck)]
            h, s = dict(K=(k_h, k_s), V=(v_h, v_s))[a]
            r = 4 * ck
            return h.at[g // hs, d, g & (hs - 1), _al((SK - WIN) // r + p, r)], s.at[g, d, _al(p, r)]

        def issue(spec, ck, size, sem, j=0, n=1, g=None, a_perm=True, pos0=None):
            per = size // ck // n
            def body(i, c):
                p = j * per + i
                if prow:
                    np_ = size // ck
                    p = (p * prow) & (np_ - 1) if a_perm else p
                pos = dict(pos0 or {})
                for t in spec.split():
                    a, cnt, prio = t[0], int(t[1:-1]), "ab".index(t[-1])
                    src, dst = views(a, pl.ds(pos.get(a, 0), cnt), p, ck, g)
                    pltpu.make_async_copy(src, dst, sem).start(priority=prio)
                    pos[a] = pos.get(a, 0) + cnt
            _loop(per, body)

        def issue_kv(g, j=0, n=1):
            issue(P3, p3[2], 256, sems.at[8 + (g & 7)], j, n, g)

        def wait(buf, sem):
            pltpu.make_async_copy(buf, buf, sem).wait()

        def head_mask():
            return (_iota((64, 1024), 0) & 15) == (_iota((64, 1024), 1) & 15)

        def w_blk(w_s, s, t):
            return w_s[s, :, _al(t, 16), :].reshape(1024, 128)

        def expand(x, u):
            return jnp.where(head_mask(), _dot(x, r_s[u]), 0.0).astype(BF)

        def head(o_s, h):
            return o_s[pl.ds(h, 4, stride=32), :]

        def project(w_s, o_s, s0, ns, j):
            l = jnp.concatenate([head(o_s, 4 * (s0 + s) + j) for s in range(ns)], axis=1).astype(BF)
            w = w_s[pl.ds(s0, ns), _al(j, 128), :].reshape(128 * ns, 512)
            return _dot(l, w)

        xcopies = [pltpu.make_async_copy(xa_h, xa_s, xsem), pltpu.make_async_copy(xb_h, xb_s, xsem)]
        if xfirst:
            for c in xcopies: c.start()
        issue(P1, p1[2], 512, sems.at[0])
        if not xfirst:
            for c in xcopies: c.start()
        issue(P2, p2[2], 512, sems.at[1], 0, 8)
        for _ in range(pad): pl.delay(1)
        for c in xcopies: c.wait()
        if on("q"):
            def rbody(i, c):
                u, r = i >> 3, i & 7
                hit = (_iota((16, 1024), 0) + 16 * r) == (_iota((16, 1024), 1) >> 4) + 64 * u
                r_s[u, _al(r, 16), :] = jnp.where(hit, 1.0, 0.0).astype(BF)
            _loop(16, rbody)
            xb = xb_s[...].astype(F32)
            for b in range(4):
                for j in range(4):
                    x64_s[j, 16 * b:16 * b + 16, :] = jnp.broadcast_to(
                        xb[b:b + 1, 128 * j:128 * j + 128], (16, 128)).astype(BF)
        issue(P2, p2[2], 512, sems.at[1], 1, 8)

        for buf in (bq_s, uk_s, wq_s, uv_s, bo_s): wait(buf, sems.at[0])
        def qb_step(s, acc):
            issue(P2, p2[2], 512, sems.at[1], 8 + s, 32)
            if not on("q"): return acc
            xe = expand(x64_s[s >> 1], s & 1)
            return tuple(acc[t] + _dot(xe, w_blk(bq_s, s, t)) for t in range(2))
        q = _loop(8, qb_step, (jnp.zeros((64, 128), F32),) * 2)
        for t in range(2):
            qb_s[t] = q[t].astype(BF)

        def ql_step(i, c):
            issue(P2, p2[2], 512, sems.at[1], 16 + i, 32)
            if not on("l"): return
            j, t = i >> 1, i & 1
            def half(u, res):
                full = _dot_nt(qb_s[t], w_blk(uk_s, 2 * j + u, t))
                sel = jnp.where(head_mask(), full, 0.0).astype(BF)
                return res + _dot_nt(sel, r_s[u])
            res = _loop(2, half, jnp.zeros((64, 128), F32)).astype(BF)
            for b in range(4):
                ql_s[b, j, _al(t, 16), :] = res[16 * b:16 * b + 16]
        _loop(8, ql_step)

        xa = xa_s[...]
        def qa_step(i, c):
            issue(P2, p2[2], 512, sems.at[1], 24 + i, 32)
            if not on("a"): return
            q = _dot(xa, wq_s[:, :, _al(i, 512)].reshape(512, 512))
            for h in range(4):
                qa_s[pl.ds(4 * i + h, 4, stride=32), :] = q[:, 128 * h:128 * h + 128]
        _loop(8, qa_step)
        issue_kv(0)

        wait(c_s, sems.at[1])
        def c_step(b, c):
            ql = jnp.concatenate([ql_s[b, j] for j in range(4)], axis=1)

            def body1(j, m):
                issue_kv(b + 1, j, 16)
                if not on("c"): return m
                s = _dot_nt(ql, c_s[8 * b + j]) * scale
                sc_s[j] = s
                return jnp.maximum(m, s)
            m = _loop(8, body1, jnp.full((32, 512), -jnp.inf, F32))
            m = jnp.max(m, axis=1, keepdims=True)

            def body2(j, carry):
                issue_kv(b + 1, 8 + j, 16)
                if not on("c"): return carry
                l, acc = carry
                p = jnp.exp(sc_s[j] - m)
                return l + p, acc + _dot(p.astype(BF), c_s[8 * b + j])
            l, acc = _loop(8, body2, (jnp.zeros((32, 512), F32),) * 2)
            cl = (acc * (1.0 / jnp.sum(l, axis=1, keepdims=True))).astype(BF)
            for j in range(4):
                for t in range(2):
                    cl_s[j, t, b] = cl[16 * t:16 * t + 16, 128 * j:128 * j + 128]
        _loop(4, c_step)

        def ctx_outer(t, c):
            def ctx_step(s, acc):
                issue_kv(5, 8 * t + s, 16)
                if not on("v"): return acc
                return acc + _dot(expand(cl_s[s >> 1, t].reshape(64, 128), s & 1), w_blk(uv_s, s, t))
            ctx = _loop(8, ctx_step, jnp.zeros((64, 128), F32))
            for b in range(4):
                ob_s[_al(2 * b + t, 16), :] = ctx[16 * b:16 * b + 16]
        _loop(2, ctx_outer)

        def ob_step(i, acc):
            issue_kv(6, i, 8)
            if not on("o"): return acc
            return acc + project(bo_s, ob_s, 4 * (i & 1), 4, i >> 1)
        out_s[:, 512:] = _loop(8, ob_step, jnp.zeros((4, 512), F32)).astype(BF)
        for _ in range(pad2): pl.delay(1)

        def stage_list():
            s0 = 0
            for k, (pat, ck) in enumerate(stages):
                segs = re.findall(r"(\d+)([ab])", pat)
                ns = sum(int(n) for n, c in segs) if segs else 1
                yield k, s0, ns, segs, pat, ck
                s0 += ns
            assert s0 == 8

        def issue_last():
            for k, s0, ns, segs, pat, ck in stage_list():
                if segs:
                    issue(" ".join(f"a{n}{c}" for n, c in segs), ck, 512, sems.at[16 + k], 3, 4, a_perm=False, pos0=dict(a=s0))
                else:
                    for i in range(128 // ck):
                        ix = (s0, pl.ds(384 + i * ck, ck))
                        pltpu.make_async_copy(wo_h.at[ix], wo_s.at[ix], sems.at[16 + k]).start(priority="ab".index(pat[i % len(pat)]))

        def kv_step(g, c):
            wait(k_s.at[g], sems.at[8 + (g & 7)])
            wait(v_s.at[g], sems.at[8 + (g & 7)])
            lo = jnp.where(g < 10, 14 + g, 2 * g + 4)
            hi = jnp.where(g < 10, 15 + g, jnp.minimum(2 * g + 6, 32))
            lax.fori_loop(lo, hi, lambda i, c: issue_kv(i >> 1, i & 1, 2), None)
            lax.fori_loop(jnp.clip(2 * g - 28, 0, 3), jnp.clip(2 * g - 26, 0, 3),
                          lambda j, c: issue(P4, p4[2], 512, sems.at[4 + j], j, 4, a_perm=False), None)
            pl.when(g == 15)(issue_last)
            if not on("k"): return
            rows = pl.ds((g // hs) * (8 * hs) + (g & (hs - 1)), 8, stride=hs)
            q = qa_s[rows, :].astype(BF)
            def qk(i, s):
                return jnp.where(_iota((8, WIN), 0) == i, _dot_nt(q, k_s[g, i]), s)
            s = _loop(8, qk, jnp.zeros((8, WIN), F32), unroll=2) * scale
            p = jnp.exp(s - jnp.max(s, axis=1, keepdims=True))
            l = jnp.sum(p, axis=1, keepdims=True)
            pb = p.astype(BF)
            def pv(i, o):
                return jnp.where(_iota((8, 128), 0) == i, _dot(pb, v_s[g, i]), o)
            oa_s[rows, :] = _loop(8, pv, jnp.zeros((8, 128), F32), unroll=2) / l
        _loop(16, kv_step)

        def out_step(j, acc):
            wait(wo_s.at[:, _al(j, 128)], sems.at[4 + j])
            if not on("w"): return acc
            return acc + project(wo_s, oa_s, 0, 8, j)
        acc = _loop(3, out_step, jnp.zeros((4, 512), F32))
        for k, s0, ns, segs, pat, ck in stage_list():
            if on("w"): l = jnp.concatenate([head(oa_s, 4 * (s0 + s) + 3) for s in range(ns)], axis=1).astype(BF)
            wait(wo_s.at[pl.ds(s0, ns), pl.ds(384, 128)], sems.at[16 + k])
            if on("w"): acc = acc + _dot(l, wo_s[s0:s0 + ns, 384:512, :].reshape(128 * ns, 512))
        out_s[:, :512] = acc.astype(BF)
        oc = pltpu.make_async_copy(out_s, out_h, xsem)
        oc.start()
        oc.wait()

    def f(A_x, A_k_cache, A_v_cache, A_wq, A_wo, B_x, B_c_kv, B_w_q, B_w_uk, B_w_uv, B_w_o):
        vm = pltpu.VMEM
        out = pl.pallas_call(
            kernel,
            out_shape=jax.ShapeDtypeStruct((4, 1024), BF),
            in_specs=[pl.BlockSpec(memory_space=pltpu.HBM)] * 11,
            out_specs=pl.BlockSpec(memory_space=pltpu.HBM),
            scratch_shapes=[
                vm((4, 512), BF), vm((16, 8, WIN, 128), BF), vm((16, 8, WIN, 128), BF),
                vm((8, 64, 4096), BF), vm((8, 512, 512), BF), vm((4, 512), BF), vm((32, 512, 512), BF),
                vm((8, 64, 32, 128), BF), vm((8, 64, 32, 128), BF), vm((8, 64, 32, 128), BF),
                vm((8, 512, 512), BF),
                vm((2, 128, 1024), BF), vm((4, 64, 128), BF), vm((2, 64, 128), BF), vm((4, 4, 32, 128), BF),
                vm((8, 32, 512), F32), vm((4, 2, 4, 16, 128), BF), vm((128, 128), F32),
                vm((128, 128), F32), vm((128, 128), F32), vm((4, 1024), BF),
                pltpu.SemaphoreType.DMA((16 + len(stages),)), pltpu.SemaphoreType.DMA,
            ],
            compiler_params=pltpu.CompilerParams(
                vmem_limit_bytes=124 << 20, disable_bounds_checks=True,
                disable_semaphore_checks=not semchecks, flags=flags),
        )(A_x.reshape(4, 512), A_k_cache.reshape(GO, 8, hs, SK, 128), A_v_cache.reshape(GO, 8, hs, SK, 128),
          A_wq.reshape(8, 64, 4096), A_wo.reshape(8, 512, 512), B_x.reshape(4, 512),
          B_c_kv.reshape(32, 512, 512), B_w_q.reshape(8, 64, 32, 128), B_w_uk.reshape(8, 64, 32, 128),
          B_w_uv.reshape(8, 64, 32, 128), B_w_o.reshape(8, 512, 512))
        return out.reshape(4, 1, 1024)
    return f


_impl = make(**dict(p1=('1a3b','x',8),p2=('4a12b','sep',8),p3=('1a3b','x',16),p4=('2a6b','sep',8),hs=2,stages=(('1a2b',16),('3b',128),('b',128),('b',128))))


@jax.jit
def pallas_concat_heads__sliding_block_cached__compressed_kv_cla__decode_kernel(
        A_x, A_k_cache, A_v_cache, A_wq, A_wo, B_x, B_c_kv, B_w_q, B_w_uk, B_w_uv, B_w_o):
    return _impl(A_x, A_k_cache, A_v_cache, A_wq, A_wo, B_x, B_c_kv, B_w_q, B_w_uk, B_w_uv, B_w_o)
```

```python
import re

import jax
import jax.numpy as jnp
from jax import lax
from jax.experimental import pallas as pl
from jax.experimental.pallas import tpu as pltpu

BF = jnp.bfloat16
F32 = jnp.float32
SK, WIN = 4096, 1024


def _dot(a, b):
    return jnp.dot(a, b, preferred_element_type=F32)


def _dot_nt(a, b):
    return lax.dot_general(a, b, (((1,), (1,)), ((), ())), preferred_element_type=F32)


def _iota(shape, dim):
    return lax.broadcasted_iota(jnp.int32, shape, dim)


def _loop(n, body, init=None, unroll=False):
    return lax.fori_loop(0, n, body, init, unroll=unroll)


def _al(i, n):
    return pl.ds(i * n if isinstance(i, int) else pl.multiple_of(i * n, n), n)


def rep(pat, names, mode="sep"):
    pp = [(int(n), c) for n, c in re.findall(r"(\d+)([ab])", pat)]
    tot = sum(n for n, _ in pp)
    out = []
    if mode == "sep":
        for a in names:
            for _ in range((32 if a == "c" else 8) // tot):
                out += [f"{a}{n}{c}" for n, c in pp]
    elif mode == "alt":
        for _ in range(8 // tot):
            for a in names:
                out += [f"{a}{n}{c}" for n, c in pp]
    else:
        m, sh = len(names), int(mode[1:] or 1)
        for _ in range(8 // tot):
            for i in range(m):
                out += [f"{names[(i + k * sh) % m]}{n}{c}" for k, (n, c) in enumerate(pp)]
    return " ".join(out)


def make(p1=("1a3b", "x", 8), p2=("4a12b", "sep", 8), p3=("1a3b", "x", 16), p4=("2a6b", "sep", 8),
         stages=(("1a2b", 16), ("3b", 128), ("1b", 128), ("1b", 128)), n1="quwvo",
         compute="all", semchecks=False, bchecks=False, flags=None, pad=0, un=2, L3=1):
    on = lambda name: compute == "all" or name in compute
    P1, P2, P3, P4 = rep(p1[0], n1, p1[1]), rep(p2[0], "c"), rep(p3[0], "KV", p3[1]), rep(p4[0], "a")
    stage_list = []
    s0 = 0
    for pat, ck in stages:
        segs = re.findall(r"(\d+)([ab])", pat)
        stage_list.append((s0, sum(int(n) for n, c in segs), " ".join(f"a{n}{c}" for n, c in segs), ck))
        s0 += stage_list[-1][1]
    assert s0 == 8

    def kernel(xa_h, k_h, v_h, wq_h, wo_h, xb_h, c_h, bq_h, uk_h, uv_h, bo_h, out_h,
               xa_s, k_s, v_s, wq_s, wo_s, xb_s, c_s, bq_s, uk_s, uv_s, bo_s,
               r_s, xa32_s, xb64_s, qb_s, ql_s, sc_s, cl_s, qa_s, oa_s, ob_s, out_s,
               w_sem, k_sem, v_sem, wo_sem, x_sem):
        scale = 128 ** -0.5

        def copy(a, d, p, ck, g):
            if a in "quv":
                h, s = dict(q=(bq_h, bq_s), u=(uk_h, uk_s), v=(uv_h, uv_s))[a]
                ix = (d, _al(p, ck // 8))
                return h.at[ix], s.at[ix], w_sem.at["quwvoc".index(a)]
            if a == "w":
                m = 64 // ck
                ix = (d, _al(p // m, 8), _al(p & (m - 1), 64 * ck))
                return wq_h.at[ix], wq_s.at[ix], w_sem.at[2]
            if a in "coa":
                h, s = dict(c=(c_h, c_s), o=(bo_h, bo_s), a=(wo_h, wo_s))[a]
                ix = (d, _al(p, ck))
                return h.at[ix], s.at[ix], (wo_sem.at[g] if a == "a" else w_sem.at["quwvoc".index(a)])
            h, s, sem = dict(K=(k_h, k_s, k_sem), V=(v_h, v_s, v_sem))[a]
            r = 4 * ck
            return h.at[g >> 1, d, g & 1, _al((SK - WIN) // r + p, r)], s.at[g, d, _al(p, r)], sem.at[g]

        def issue(spec, ck, size, j=0, n=1, g=None, first=0, L=1):
            per = size // ck // n
            items = spec.split()
            step = 2 if L > 1 else len(items)
            def body(i, c):
                pos0 = {}
                for k0 in range(0, len(items), step):
                    for l in range(L):
                        pos = dict(pos0)
                        for t in items[k0:k0 + step]:
                            a, cnt, prio = t[0], int(t[1:-1]), "ab".index(t[-1])
                            s0 = pos.get(a, first)
                            pltpu.make_async_copy(*copy(a, pl.ds(s0, cnt), j * per + i * L + l, ck, g)).start(priority=prio)
                            pos[a] = s0 + cnt
                    pos0 = pos
            if per == 1:
                body(0, None)
            else:
                _loop(per // L, body)

        issue_c = lambda j, n: issue(P2, p2[2], 512, j, n)
        issue_kv = lambda g, j=0, n=1: issue(P3, p3[2], 256, j, n, g, L=L3)

        def wait(buf, sem):
            pltpu.make_async_copy(buf, buf, sem).wait()

        def head_mask():
            return (_iota((64, 1024), 0) & 15) == (_iota((64, 1024), 1) & 15)

        def w_blk(w_s, s, t):
            return w_s[s, :, _al(t, 16), :].reshape(1024, 128)

        def expand(x, u):
            return jnp.where(head_mask(), _dot(x, r_s[u]), 0.0).astype(BF)

        def heads(o_s, s0, ns, j):
            return jnp.concatenate([o_s[4 * (s0 + s) + j] for s in range(ns)], axis=1).astype(BF)

        def w_rows(w_s, s0, ns, j):
            return w_s[pl.ds(s0, ns), _al(j, 128), :].reshape(128 * ns, 512)

        x_copies = [pltpu.make_async_copy(xa_h, xa_s, x_sem.at[0]), pltpu.make_async_copy(xb_h, xb_s, x_sem.at[1])]
        issue(P1, p1[2], 512)
        for cp in x_copies:
            cp.start()
        issue_c(0, 8)
        for cp in x_copies:
            cp.wait()

        def r_step(i, c):
            u, r = i >> 3, i & 7
            hit = (_iota((16, 1024), 0) + 16 * r) == (_iota((16, 1024), 1) >> 4) + 64 * u
            r_s[u, _al(r, 16), :] = jnp.where(hit, 1.0, 0.0).astype(BF)
        _loop(16, r_step)
        xa, xb = xa_s[...].astype(F32), xb_s[...].astype(F32)
        xa32_s[...] = jnp.concatenate([jnp.broadcast_to(xa[b:b + 1], (8, 512)) for b in range(4)], axis=0).astype(BF)
        for b in range(4):
            for j in range(4):
                xb64_s[j, 16 * b:16 * b + 16, :] = jnp.broadcast_to(
                    xb[b:b + 1, 128 * j:128 * j + 128], (16, 128)).astype(BF)
        oa_s[...] = jnp.zeros(oa_s.shape, F32)
        issue_c(1, 8)
        for i, buf in enumerate((bq_s, uk_s, wq_s, uv_s, bo_s)):
            wait(buf, w_sem.at[i])

        def qb_step(s, acc):
            issue_c(8 + s, 32)
            if not on("q"): return acc
            xe = expand(xb64_s[s >> 1], s & 1)
            return tuple(acc[t] + _dot(xe, w_blk(bq_s, s, t)) for t in range(2))
        q = _loop(8, qb_step, (jnp.zeros((64, 128), F32),) * 2)
        for t in range(2):
            qb_s[t] = q[t].astype(BF)

        def ql_step(i, c):
            issue_c(16 + i, 32)
            if not on("l"): return
            j, t = i >> 1, i & 1
            def half(u, res):
                full = _dot_nt(qb_s[t], w_blk(uk_s, 2 * j + u, t))
                return res + _dot_nt(jnp.where(head_mask(), full, 0.0).astype(BF), r_s[u])
            res = _loop(2, half, jnp.zeros((64, 128), F32)).astype(BF)
            for b in range(4):
                ql_s[b, j, _al(t, 16), :] = res[16 * b:16 * b + 16]
        _loop(8, ql_step)

        def qa_step(i, c):
            issue_c(24 + i, 32)
            if not on("a"): return
            q = _dot(xa32_s[...], wq_s[:, :, _al(i, 512)].reshape(512, 512))
            for h in range(4):
                qa_s[4 * i + h] = q[:, 128 * h:128 * h + 128]
        _loop(8, qa_step)
        issue_kv(0)

        wait(c_s, w_sem.at[5])
        def c_step(b, c):
            ql = jnp.concatenate([ql_s[b, j] for j in range(4)], axis=1)

            def score(j, m):
                issue_kv(b + 1, j, 16) if L3 == 1 else issue_kv(b + 1, j, 16)
                if not on("c"): return m
                s = _dot_nt(ql, c_s[8 * b + j]) * scale
                sc_s[j] = s
                return jnp.maximum(m, s)
            m = _loop(8, score, jnp.full((32, 512), -jnp.inf, F32))
            m = jnp.max(m, axis=1, keepdims=True)

            def mix(j, carry):
                issue_kv(b + 1, 8 + j, 16)
                if not on("c"): return carry
                l, acc = carry
                p = jnp.exp(sc_s[j] - m)
                return l + p, acc + _dot(p.astype(BF), c_s[8 * b + j])
            l, acc = _loop(8, mix, (jnp.zeros((32, 512), F32),) * 2)
            cl = (acc / jnp.sum(l, axis=1, keepdims=True)).astype(BF)
            for j in range(4):
                for t in range(2):
                    cl_s[j, t, _al(b, 16), :] = cl[16 * t:16 * t + 16, 128 * j:128 * j + 128]
        _loop(4, c_step)

        def ctx_half(t, c):
            def ctx_step(s, acc):
                issue_kv(5, 8 * t + s, 16)
                if not on("v"): return acc
                return acc + _dot(expand(cl_s[s >> 1, t], s & 1), w_blk(uv_s, s, t))
            ctx = _loop(8, ctx_step, jnp.zeros((64, 128), F32))
            row = _iota((8, 128), 0)
            for h in range(16):
                o = jnp.zeros((8, 128), F32)
                for b in range(4):
                    o = jnp.where(row == b, ctx[16 * b + h:16 * b + h + 1], o)
                ob_s[16 * t + h] = o
        _loop(2, ctx_half)

        def ob_step(i, acc):
            issue_kv(6, i, 8)
            if not on("o"): return acc
            s0, j = 4 * (i & 1), i >> 1
            return acc + _dot(heads(ob_s, s0, 4, j), w_rows(bo_s, s0, 4, j))
        out_s[:, 512:] = _loop(8, ob_step, jnp.zeros((8, 512), F32))[:4].astype(BF)
        for _ in range(pad): pl.delay(1)

        def kv_step(g, c):
            wait(k_s.at[g], k_sem.at[g])
            wait(v_s.at[g], v_sem.at[g])
            lax.fori_loop(jnp.where(g < 10, 14 + g, 2 * g + 4),
                          jnp.where(g < 10, 15 + g, jnp.minimum(2 * g + 6, 32)),
                          lambda i, c: issue_kv(i >> 1, i & 1, 2), None)
            lax.fori_loop(jnp.clip(2 * g - 28, 0, 3), jnp.clip(2 * g - 26, 0, 3),
                          lambda j, c: issue(P4, p4[2], 512, j, 4, j), None)
            if not on("k"): return
            b, h0 = g >> 2, 16 * ((g >> 1) & 1) + (g & 1)

            def qk(i, s):
                q = qa_s[h0 + 2 * i, _al(b, 8), :].astype(BF)
                return jnp.where(_iota((8, WIN), 0) == i, _dot_nt(q, k_s[g, i]), s)
            s = _loop(8, qk, jnp.zeros((8, WIN), F32), unroll=un) * scale
            p = jnp.exp(s - jnp.max(s, axis=1, keepdims=True))
            pb = p.astype(BF)

            def pv(i, o):
                return jnp.where(_iota((8, 128), 0) == i, _dot(pb, v_s[g, i]), o)
            o = _loop(8, pv, jnp.zeros((8, 128), F32), unroll=un) / jnp.sum(p, axis=1, keepdims=True)
            for i in range(8):
                oa_s[h0 + 2 * i] = jnp.where(_iota((8, 128), 0) == b, o[i:i + 1], oa_s[h0 + 2 * i])
        _loop(16, kv_step)

        for k, (s0, ns, spec, ck) in enumerate(stage_list):
            issue(spec, ck, 512, 3, 4, 3 + k, s0)

        def oa_step(j, acc):
            wait(wo_s.at[:, _al(j, 128)], wo_sem.at[j])
            if not on("w"): return acc
            return acc + _dot(heads(oa_s, 0, 8, j), w_rows(wo_s, 0, 8, j))
        acc = _loop(3, oa_step, jnp.zeros((8, 512), F32))
        for k, (s0, ns, spec, ck) in enumerate(stage_list):
            lhs = heads(oa_s, s0, ns, 3)
            wait(wo_s.at[pl.ds(s0, ns), pl.ds(384, 128)], wo_sem.at[3 + k])
            if on("w"): acc = acc + _dot(lhs, w_rows(wo_s, s0, ns, 3))
        out_s[:, :512] = acc[:4].astype(BF)
        out_copy = pltpu.make_async_copy(out_s, out_h, x_sem.at[2])
        out_copy.start()
        out_copy.wait()

    def f(A_x, A_k_cache, A_v_cache, A_wq, A_wo, B_x, B_c_kv, B_w_q, B_w_uk, B_w_uv, B_w_o):
        vm, dma = pltpu.VMEM, pltpu.SemaphoreType.DMA
        out = pl.pallas_call(
            kernel,
            out_shape=jax.ShapeDtypeStruct((4, 1024), BF),
            in_specs=[pl.BlockSpec(memory_space=pltpu.HBM)] * 11,
            out_specs=pl.BlockSpec(memory_space=pltpu.HBM),
            scratch_shapes=[
                vm((4, 512), BF), vm((16, 8, WIN, 128), BF), vm((16, 8, WIN, 128), BF),
                vm((8, 64, 4096), BF), vm((8, 512, 512), BF), vm((4, 512), BF), vm((32, 512, 512), BF),
                vm((8, 64, 32, 128), BF), vm((8, 64, 32, 128), BF), vm((8, 64, 32, 128), BF),
                vm((8, 512, 512), BF),
                vm((2, 128, 1024), BF), vm((32, 512), BF), vm((4, 64, 128), BF), vm((2, 64, 128), BF),
                vm((4, 4, 32, 128), BF), vm((8, 32, 512), F32), vm((4, 2, 64, 128), BF),
                vm((32, 32, 128), F32), vm((32, 8, 128), F32), vm((32, 8, 128), F32), vm((4, 1024), BF),
                dma((6,)), dma((16,)), dma((16,)), dma((3 + len(stages),)), dma((3,)),
            ],
            compiler_params=pltpu.CompilerParams(
                vmem_limit_bytes=120 << 20, disable_bounds_checks=not bchecks,
                disable_semaphore_checks=not semchecks, flags=flags),
        )(A_x.reshape(4, 512), A_k_cache.reshape(8, 8, 2, SK, 128), A_v_cache.reshape(8, 8, 2, SK, 128),
          A_wq.reshape(8, 64, 4096), A_wo.reshape(8, 512, 512), B_x.reshape(4, 512),
          B_c_kv.reshape(32, 512, 512), B_w_q.reshape(8, 64, 32, 128), B_w_uk.reshape(8, 64, 32, 128),
          B_w_uv.reshape(8, 64, 32, 128), B_w_o.reshape(8, 512, 512))
        return out.reshape(4, 1, 1024)
    return f


_impl = make(**dict())


@jax.jit
def pallas_concat_heads__sliding_block_cached__compressed_kv_cla__decode_kernel(
        A_x, A_k_cache, A_v_cache, A_wq, A_wo, B_x, B_c_kv, B_w_q, B_w_uk, B_w_uv, B_w_o):
    return _impl(A_x, A_k_cache, A_v_cache, A_wq, A_wo, B_x, B_c_kv, B_w_q, B_w_uk, B_w_uv, B_w_o)
```

```python
import jax
import jax.numpy as jnp
from jax import lax
from jax.experimental import pallas as pl
from jax.experimental.pallas import tpu as pltpu

BF16 = jnp.bfloat16
F32 = jnp.float32

SK = 4096
WIN = min(4096, max(256, SK // 4))
SCALE = 128 ** -0.5

WO_TAIL = ((0, ((1, 0), (3, 1)), 16), (4, ((2, 1),), 16), (6, ((1, 1),), 128), (7, ((1, 1),), 128))


def _dot(a, b):
    return jnp.dot(a, b, preferred_element_type=F32)


def _dot_nt(a, b):
    return lax.dot_general(a, b, (((1,), (1,)), ((), ())), preferred_element_type=F32)


def _iota(shape, dim):
    return lax.broadcasted_iota(jnp.int32, shape, dim)


def _loop(n, body, init=None, unroll=False):
    return lax.fori_loop(0, n, body, init, unroll=unroll)


def _blk(i, n):
    return pl.ds(i * n if isinstance(i, int) else pl.multiple_of(i * n, n), n)


def _kernel(
    xa_h,
    k_h,
    v_h,
    wq_h,
    wo_h,
    xb_h,
    c_h,
    bq_h,
    uk_h,
    uv_h,
    bo_h,
    out_h,
    xa_s, k_s, v_s, wq_s, wo_s, xb_s, c_s, bq_s, uk_s, uv_s, bo_s,
    rep_s,
    xa8_s,
    xb16_s,
    qb_s,
    ql_s,
    sc_s,
    cl_s,
    qa_s,
    oa_s,
    ob_s,
    out_s,
    w_sem, k_sem, v_sem, wo_sem, x_sem,
):
    def start(src, dst, sem, thread):
        pltpu.make_async_copy(src, dst, sem).start(priority=thread)

    def wait_filled(buf, sem):
        pltpu.make_async_copy(buf, buf, sem).wait()

    def weight_row(p, carry):
        piece = (_blk(p, 1),)
        arrays = (
            (bq_h, bq_s, piece),
            (uk_h, uk_s, piece),
            (wq_h, wq_s, (_blk(p >> 3, 8), _blk(p & 7, 512))),
            (uv_h, uv_s, piece),
            (bo_h, bo_s, (_blk(p, 8),)),
        )
        for i, (src, dst, ix) in enumerate(arrays):
            for streams, thread in ((pl.ds(0, 1), 0), (pl.ds(1, 3), 1)):
                start(src.at[(streams,) + ix], dst.at[(streams,) + ix], w_sem.at[i], thread)

    def issue_c(part, parts):
        rows = 128 // parts

        def row(i, carry):
            for half in range(2):
                for streams, thread in ((pl.ds(0, 1), 0), (pl.ds(1, 7), 1)):
                    ix = (streams, half, _blk(part * rows + i, 8))
                    start(c_h.at[ix], c_s.at[ix], w_sem.at[5], thread)
        _loop(rows, row)

    def issue_kv(g, part=0, parts=1):
        rows = WIN // 64 // parts
        k, v = (k_h, k_s, k_sem), (v_h, v_s, v_sem)

        def row(i, carry):
            p = part * rows + i
            for s0 in (0, 4):
                for first, second in ((k, v), (v, k)):
                    for (src, dst, sem), streams, thread in (
                            (first, pl.ds(s0, 1), 0), (second, pl.ds(s0 + 1, 3), 1)):
                        start(src.at[g >> 1, streams, g & 1, _blk((SK - WIN) // 64 + p, 64)],
                              dst.at[g, streams, _blk(p, 64)], sem.at[g], thread)
        if rows == 1:
            row(0, None)
        else:
            _loop(rows, row)

    def issue_wo(quarter, sem, first, segments, rows):
        def row(i, carry):
            s0 = first
            for n, thread in segments:
                ix = (pl.ds(s0, n), _blk(quarter * (128 // rows) + i, rows))
                start(wo_h.at[ix], wo_s.at[ix], sem, thread)
                s0 += n
        if rows == 128:
            row(0, None)
        else:
            _loop(128 // rows, row)

    def same_head():
        return (_iota((64, 1024), 0) & 15) == (_iota((64, 1024), 1) & 15)

    def w_block(w_s, s, t):
        return w_s[s >> 1, _blk(s & 1, 64), _blk(t, 16), :].reshape(1024, 128)

    def head_diagonal(x, u):
        return jnp.where(same_head(), _dot(x, rep_s[u]), 0.0).astype(BF16)

    def project_a(s0, n, quarter, sem):
        lhs = jnp.concatenate([oa_s[4 * (s0 + s) + quarter] for s in range(n)], axis=1).astype(BF16)
        ix = (pl.ds(s0, n), _blk(quarter, 128))
        wait_filled(wo_s.at[ix], sem)
        return _dot(lhs, wo_s[ix].reshape(128 * n, 512))

    x_copies = [pltpu.make_async_copy(xa_h, xa_s, x_sem.at[0]),
                pltpu.make_async_copy(xb_h, xb_s, x_sem.at[1])]
    _loop(128, weight_row)
    for copy in x_copies:
        copy.start()
    issue_c(0, 8)
    for copy in x_copies:
        copy.wait()

    def rep_step(i, carry):
        u, r = i >> 3, i & 7
        hit = _iota((16, 1024), 0) + 16 * r == (_iota((16, 1024), 1) >> 4) + 64 * u
        rep_s[u, _blk(r, 16), :] = jnp.where(hit, 1.0, 0.0).astype(BF16)
    _loop(16, rep_step)
    xa, xb = xa_s[...].astype(F32), xb_s[...].astype(F32)
    xa8_s[...] = jnp.concatenate(
        [jnp.broadcast_to(xa[b:b + 1], (8, 512)) for b in range(4)], axis=0).astype(BF16)
    for b in range(4):
        for j in range(4):
            xb16_s[j, 16 * b:16 * b + 16, :] = jnp.broadcast_to(
                xb[b:b + 1, 128 * j:128 * j + 128], (16, 128)).astype(BF16)
    oa_s[...] = jnp.zeros(oa_s.shape, F32)
    issue_c(1, 8)
    for i, buf in enumerate((bq_s, uk_s, wq_s, uv_s, bo_s)):
        wait_filled(buf, w_sem.at[i])

    def qb_step(s, acc):
        issue_c(8 + s, 32)
        x = head_diagonal(xb16_s[s >> 1], s & 1)
        return tuple(acc[t] + _dot(x, w_block(bq_s, s, t)) for t in range(2))
    qb = _loop(8, qb_step, (jnp.zeros((64, 128), F32),) * 2)
    for t in range(2):
        qb_s[t] = qb[t].astype(BF16)

    def ql_step(i, carry):
        issue_c(16 + i, 32)
        j, t = i >> 1, i & 1

        def half(u, acc):
            every_pair = _dot_nt(qb_s[t], w_block(uk_s, 2 * j + u, t))
            return acc + _dot_nt(jnp.where(same_head(), every_pair, 0.0).astype(BF16), rep_s[u])
        ql = _loop(2, half, jnp.zeros((64, 128), F32)).astype(BF16)
        for b in range(4):
            ql_s[b, j, _blk(t, 16), :] = ql[16 * b:16 * b + 16]
    _loop(8, ql_step)

    def qa_step(i, carry):
        issue_c(24 + i, 32)
        q = _dot(xa8_s[...], wq_s[:, :, _blk(i, 512)].reshape(512, 512))
        for h in range(4):
            qa_s[4 * i + h] = q[:, 128 * h:128 * h + 128]
    _loop(8, qa_step)

    issue_kv(0)
    wait_filled(c_s, w_sem.at[5])

    def latent_step(b, carry):
        ql = jnp.concatenate([ql_s[b, j] for j in range(4)], axis=1)

        def keys(j):
            return c_s[2 * b + (j >> 2), (j >> 1) & 1, _blk(j & 1, 512), :]

        def score(j, m):
            issue_kv(b + 1, j, 16)
            s = _dot_nt(ql, keys(j)) * SCALE
            sc_s[j] = s
            return jnp.maximum(m, s)
        m = _loop(8, score, jnp.full((32, 512), -jnp.inf, F32))
        m = jnp.max(m, axis=1, keepdims=True)

        def mix(j, sums):
            issue_kv(b + 1, 8 + j, 16)
            p = jnp.exp(sc_s[j] - m)
            return sums[0] + p, sums[1] + _dot(p.astype(BF16), keys(j))
        l, acc = _loop(8, mix, (jnp.zeros((32, 512), F32),) * 2)
        cl = (acc / jnp.sum(l, axis=1, keepdims=True)).astype(BF16)
        for j in range(4):
            for t in range(2):
                cl_s[j, t, _blk(b, 16), :] = cl[16 * t:16 * t + 16, 128 * j:128 * j + 128]
    _loop(4, latent_step)

    def context_half(t, carry):
        def step(s, acc):
            issue_kv(5, 8 * t + s, 16)
            return acc + _dot(head_diagonal(cl_s[s >> 1, t], s & 1), w_block(uv_s, s, t))
        ctx = _loop(8, step, jnp.zeros((64, 128), F32))
        for h in range(16):
            o = jnp.zeros((8, 128), F32)
            for b in range(4):
                o = jnp.where(_iota((8, 128), 0) == b, ctx[16 * b + h:16 * b + h + 1], o)
            ob_s[16 * t + h] = o
    _loop(2, context_half)

    def out_b_step(i, acc):
        issue_kv(6, i, 8)
        lhs = jnp.concatenate([ob_s[4 * i + h] for h in range(4)], axis=1).astype(BF16)
        return acc + _dot(lhs, bo_s[i >> 1, _blk(i & 1, 512), :])
    out_s[:, 512:] = _loop(8, out_b_step, jnp.zeros((8, 512), F32))[:4].astype(BF16)

    def window_step(g, carry):
        wait_filled(k_s.at[g], k_sem.at[g])
        wait_filled(v_s.at[g], v_sem.at[g])
        lax.fori_loop(jnp.where(g < 10, g + 14, 2 * g + 4),
                      jnp.where(g < 10, g + 15, jnp.minimum(2 * g + 6, 32)),
                      lambda i, c: issue_kv(i >> 1, i & 1, 2), None)
        lax.fori_loop(jnp.clip(2 * g - 28, 0, 3), jnp.clip(2 * g - 26, 0, 3),
                      lambda j, c: issue_wo(j, wo_sem.at[j], 0, ((1, 0), (3, 1)) * 2, 16), None)
        b, h0 = g >> 2, 16 * ((g >> 1) & 1) + (g & 1)

        def score(i, s):
            q = qa_s[h0 + 2 * i, _blk(b, 8), :].astype(BF16)
            return jnp.where(_iota((8, WIN), 0) == i, _dot_nt(q, k_s[g, i]), s)
        s = _loop(8, score, jnp.zeros((8, WIN), F32), unroll=4) * SCALE
        p = jnp.exp(s - jnp.max(s, axis=1, keepdims=True))
        p16 = p.astype(BF16)

        def mix(i, o):
            return jnp.where(_iota((8, 128), 0) == i, _dot(p16, v_s[g, i]), o)
        o = _loop(8, mix, jnp.zeros((8, 128), F32), unroll=4) / jnp.sum(p, axis=1, keepdims=True)
        for i in range(8):
            oa_s[h0 + 2 * i] = jnp.where(_iota((8, 128), 0) == b, o[i:i + 1], oa_s[h0 + 2 * i])
    _loop(16, window_step)

    for i, (first, segments, rows) in enumerate(WO_TAIL):
        issue_wo(3, wo_sem.at[3 + i], first, segments, rows)
    acc = _loop(3, lambda j, acc: acc + project_a(0, 8, j, wo_sem.at[j]), jnp.zeros((8, 512), F32))
    for i, (first, segments, _) in enumerate(WO_TAIL):
        acc = acc + project_a(first, sum(n for n, _ in segments), 3, wo_sem.at[3 + i])
    out_s[:, :512] = acc[:4].astype(BF16)
    out_copy = pltpu.make_async_copy(out_s, out_h, x_sem.at[2])
    out_copy.start()
    out_copy.wait()


@jax.jit
def pallas_concat_heads__sliding_block_cached__compressed_kv_cla__decode_kernel(
    A_x: jax.Array,
    A_k_cache: jax.Array,
    A_v_cache: jax.Array,
    A_wq: jax.Array,
    A_wo: jax.Array,
    B_x: jax.Array,
    B_c_kv: jax.Array,
    B_w_q: jax.Array,
    B_w_uk: jax.Array,
    B_w_uv: jax.Array,
    B_w_o: jax.Array,
):
    operands = (
        A_x.reshape(4, 512),
        A_k_cache.reshape(8, 8, 2, SK, 128),
        A_v_cache.reshape(8, 8, 2, SK, 128),
        A_wq.reshape(4, 128, 4096),
        A_wo.reshape(8, 512, 512),
        B_x.reshape(4, 512),
        B_c_kv.reshape(8, 2, 1024, 512),
        B_w_q.reshape(4, 128, 32, 128),
        B_w_uk.reshape(4, 128, 32, 128),
        B_w_uv.reshape(4, 128, 32, 128),
        B_w_o.reshape(4, 1024, 512),
    )
    landing = [x.shape for x in operands]
    landing[1] = landing[2] = (16, 8, WIN, 128)
    vmem, dma = pltpu.VMEM, pltpu.SemaphoreType.DMA
    out = pl.pallas_call(
        _kernel,
        out_shape=jax.ShapeDtypeStruct((4, 1024), BF16),
        in_specs=[pl.BlockSpec(memory_space=pltpu.HBM)] * len(operands),
        out_specs=pl.BlockSpec(memory_space=pltpu.HBM),
        scratch_shapes=[
            *(vmem(shape, BF16) for shape in landing),
            vmem((2, 128, 1024), BF16),
            vmem((32, 512), BF16),
            vmem((4, 64, 128), BF16),
            vmem((2, 64, 128), BF16),
            vmem((4, 4, 32, 128), BF16),
            vmem((8, 32, 512), F32),
            vmem((4, 2, 64, 128), BF16),
            vmem((32, 32, 128), F32),
            vmem((32, 8, 128), F32),
            vmem((32, 8, 128), F32),
            vmem((4, 1024), BF16),
            dma((6,)), dma((16,)), dma((16,)), dma((3 + len(WO_TAIL),)), dma((3,)),
        ],
        compiler_params=pltpu.CompilerParams(
            vmem_limit_bytes=120 * 1024 * 1024,
            disable_bounds_checks=True,
            disable_semaphore_checks=True,
        ),
    )(*operands)
    return out.reshape(4, 1, 1024)
```

```python
import jax
import jax.numpy as jnp
from jax import lax
from jax.experimental import pallas as pl
from jax.experimental.pallas import tpu as pltpu

BF16 = jnp.bfloat16
F32 = jnp.float32

SK = 4096
WIN = min(4096, max(256, SK // 4))
SCALE = 128 ** -0.5

WEIGHT_ROW = (("bo", 0, 1, 0), ("wq", 0, 3, 1), ("uv", 0, 1, 0), ("uk", 0, 3, 1), ("uk", 3, 1, 0),
              ("uv", 1, 3, 1), ("bq", 3, 1, 0), ("bo", 1, 3, 1), ("wq", 3, 1, 0), ("bq", 0, 3, 1))
LATENT_ROW = (("c0", 0, 1, 0), ("c0", 1, 7, 1), ("c1", 0, 1, 0), ("c1", 1, 7, 1))
WINDOW_ROW = (("k", 0, 1, 0), ("v", 0, 3, 1), ("v", 3, 1, 0), ("k", 1, 3, 1),
              ("k", 4, 1, 0), ("v", 4, 3, 1), ("v", 7, 1, 0), ("k", 5, 3, 1))
WO_TAIL = ((0, ((1, 0), (3, 1)), 16), (4, ((2, 1),), 16), (6, ((1, 1),), 128), (7, ((1, 1),), 128))


def _dot(a, b):
    return jnp.dot(a, b, preferred_element_type=F32)


def _dot_nt(a, b):
    return lax.dot_general(a, b, (((1,), (1,)), ((), ())), preferred_element_type=F32)


def _iota(shape, dim):
    return lax.broadcasted_iota(jnp.int32, shape, dim)


def _loop(n, body, init=None, unroll=False):
    return lax.fori_loop(0, n, body, init, unroll=unroll)


def _blk(i, n):
    return pl.ds(i * n if isinstance(i, int) else pl.multiple_of(i * n, n), n)


def _kernel(
    xa_h,
    k_h,
    v_h,
    wq_h,
    wo_h,
    xb_h,
    c_h,
    bq_h,
    uk_h,
    uv_h,
    bo_h,
    out_h,
    xa_s, k_s, v_s, wq_s, wo_s, xb_s, c_s, bq_s, uk_s, uv_s, bo_s,
    rep_s,
    xa8_s,
    xb16_s,
    qb_s,
    ql_s,
    sc_s,
    cl_s,
    qa_s,
    oa_s,
    ob_s,
    out_s,
    w_sem, k_sem, v_sem, wo_sem, x_sem,
):
    def start(src, dst, sem, thread):
        pltpu.make_async_copy(src, dst, sem).start(priority=thread)

    def wait_filled(buf, sem):
        pltpu.make_async_copy(buf, buf, sem).wait()

    def contiguous_row(row, p):
        arrays = {
            "bq": (bq_h, bq_s, 0, (_blk(p, 1),)),
            "uk": (uk_h, uk_s, 1, (_blk(p, 1),)),
            "wq": (wq_h, wq_s, 2, (_blk(p >> 3, 8), _blk(p & 7, 512))),
            "uv": (uv_h, uv_s, 3, (_blk(p, 1),)),
            "bo": (bo_h, bo_s, 4, (_blk(p, 8),)),
            "c0": (c_h, c_s, 5, (0, _blk(p, 8))),
            "c1": (c_h, c_s, 5, (1, _blk(p, 8))),
        }
        for name, first, n, thread in row:
            src, dst, sem, piece = arrays[name]
            ix = (pl.ds(first, n),) + piece
            start(src.at[ix], dst.at[ix], w_sem.at[sem], thread)

    def issue_c(part, parts):
        rows = 128 // parts
        _loop(rows, lambda i, carry: contiguous_row(LATENT_ROW, part * rows + i))

    def issue_kv(g, part=0, parts=1):
        rows = WIN // 64 // parts
        arrays = {"k": (k_h, k_s, k_sem), "v": (v_h, v_s, v_sem)}

        def row(i, carry):
            p = part * rows + i
            for name, first, n, thread in WINDOW_ROW:
                src, dst, sem = arrays[name]
                start(src.at[g >> 1, pl.ds(first, n), g & 1, _blk((SK - WIN) // 64 + p, 64)],
                      dst.at[g, pl.ds(first, n), _blk(p, 64)], sem.at[g], thread)
        if rows == 1:
            row(0, None)
        else:
            _loop(rows, row)

    def issue_wo(quarter, sem, first, segments, rows):
        def row(i, carry):
            s0 = first
            for n, thread in segments:
                ix = (pl.ds(s0, n), _blk(quarter * (128 // rows) + i, rows))
                start(wo_h.at[ix], wo_s.at[ix], sem, thread)
                s0 += n
        if rows == 128:
            row(0, None)
        else:
            _loop(128 // rows, row)

    def same_head():
        return (_iota((64, 1024), 0) & 15) == (_iota((64, 1024), 1) & 15)

    def w_block(w_s, s, t):
        return w_s[s >> 1, _blk(s & 1, 64), _blk(t, 16), :].reshape(1024, 128)

    def head_diagonal(x, u):
        return jnp.where(same_head(), _dot(x, rep_s[u]), 0.0).astype(BF16)

    def project_a(s0, n, quarter, sem):
        lhs = jnp.concatenate([oa_s[4 * (s0 + s) + quarter] for s in range(n)], axis=1).astype(BF16)
        ix = (pl.ds(s0, n), _blk(quarter, 128))
        wait_filled(wo_s.at[ix], sem)
        return _dot(lhs, wo_s[ix].reshape(128 * n, 512))

    x_copies = [pltpu.make_async_copy(xa_h, xa_s, x_sem.at[0]),
                pltpu.make_async_copy(xb_h, xb_s, x_sem.at[1])]
    _loop(128, lambda p, carry: contiguous_row(WEIGHT_ROW, p))
    for copy in x_copies:
        copy.start()
    issue_c(0, 8)
    for copy in x_copies:
        copy.wait()

    def rep_step(i, carry):
        u, r = i >> 3, i & 7
        hit = _iota((16, 1024), 0) + 16 * r == (_iota((16, 1024), 1) >> 4) + 64 * u
        rep_s[u, _blk(r, 16), :] = jnp.where(hit, 1.0, 0.0).astype(BF16)
    _loop(16, rep_step)
    xa, xb = xa_s[...].astype(F32), xb_s[...].astype(F32)
    xa8_s[...] = jnp.concatenate(
        [jnp.broadcast_to(xa[b:b + 1], (8, 512)) for b in range(4)], axis=0).astype(BF16)
    for b in range(4):
        for j in range(4):
            xb16_s[j, 16 * b:16 * b + 16, :] = jnp.broadcast_to(
                xb[b:b + 1, 128 * j:128 * j + 128], (16, 128)).astype(BF16)
    oa_s[...] = jnp.zeros(oa_s.shape, F32)
    issue_c(1, 8)
    for i, buf in enumerate((bq_s, uk_s, wq_s, uv_s, bo_s)):
        wait_filled(buf, w_sem.at[i])

    def qb_step(s, acc):
        issue_c(8 + s, 32)
        x = head_diagonal(xb16_s[s >> 1], s & 1)
        return tuple(acc[t] + _dot(x, w_block(bq_s, s, t)) for t in range(2))
    qb = _loop(8, qb_step, (jnp.zeros((64, 128), F32),) * 2)
    for t in range(2):
        qb_s[t] = qb[t].astype(BF16)

    def ql_step(i, carry):
        issue_c(16 + i, 32)
        j, t = i >> 1, i & 1

        def half(u, acc):
            every_pair = _dot_nt(qb_s[t], w_block(uk_s, 2 * j + u, t))
            return acc + _dot_nt(jnp.where(same_head(), every_pair, 0.0).astype(BF16), rep_s[u])
        ql = _loop(2, half, jnp.zeros((64, 128), F32)).astype(BF16)
        for b in range(4):
            ql_s[b, j, _blk(t, 16), :] = ql[16 * b:16 * b + 16]
    _loop(8, ql_step)

    def qa_step(i, carry):
        issue_c(24 + i, 32)
        q = _dot(xa8_s[...], wq_s[:, :, _blk(i, 512)].reshape(512, 512))
        for h in range(4):
            qa_s[4 * i + h] = q[:, 128 * h:128 * h + 128]
    _loop(8, qa_step)

    issue_kv(0)
    wait_filled(c_s, w_sem.at[5])

    def latent_step(b, carry):
        ql = jnp.concatenate([ql_s[b, j] for j in range(4)], axis=1)

        def keys(j):
            return c_s[2 * b + (j >> 2), (j >> 1) & 1, _blk(j & 1, 512), :]

        def score(j, m):
            issue_kv(b + 1, j, 16)
            s = _dot_nt(ql, keys(j)) * SCALE
            sc_s[j] = s
            return jnp.maximum(m, s)
        m = _loop(8, score, jnp.full((32, 512), -jnp.inf, F32))
        m = jnp.max(m, axis=1, keepdims=True)

        def mix(j, sums):
            issue_kv(b + 1, 8 + j, 16)
            p = jnp.exp(sc_s[j] - m)
            return sums[0] + p, sums[1] + _dot(p.astype(BF16), keys(j))
        l, acc = _loop(8, mix, (jnp.zeros((32, 512), F32),) * 2)
        cl = (acc / jnp.sum(l, axis=1, keepdims=True)).astype(BF16)
        for j in range(4):
            for t in range(2):
                cl_s[j, t, _blk(b, 16), :] = cl[16 * t:16 * t + 16, 128 * j:128 * j + 128]
    _loop(4, latent_step)

    def context_half(t, carry):
        def step(s, acc):
            issue_kv(5, 8 * t + s, 16)
            return acc + _dot(head_diagonal(cl_s[s >> 1, t], s & 1), w_block(uv_s, s, t))
        ctx = _loop(8, step, jnp.zeros((64, 128), F32))
        for h in range(16):
            o = jnp.zeros((8, 128), F32)
            for b in range(4):
                o = jnp.where(_iota((8, 128), 0) == b, ctx[16 * b + h:16 * b + h + 1], o)
            ob_s[16 * t + h] = o
    _loop(2, context_half)

    def out_b_step(i, acc):
        issue_kv(6, i, 8)
        lhs = jnp.concatenate([ob_s[4 * i + h] for h in range(4)], axis=1).astype(BF16)
        return acc + _dot(lhs, bo_s[i >> 1, _blk(i & 1, 512), :])
    out_s[:, 512:] = _loop(8, out_b_step, jnp.zeros((8, 512), F32))[:4].astype(BF16)

    def window_step(g, carry):
        wait_filled(k_s.at[g], k_sem.at[g])
        wait_filled(v_s.at[g], v_sem.at[g])
        lax.fori_loop(jnp.where(g < 10, g + 14, 2 * g + 4),
                      jnp.where(g < 10, g + 15, jnp.minimum(2 * g + 6, 32)),
                      lambda i, c: issue_kv(i >> 1, i & 1, 2), None)
        lax.fori_loop(jnp.clip(2 * g - 28, 0, 3), jnp.clip(2 * g - 26, 0, 3),
                      lambda j, c: issue_wo(j, wo_sem.at[j], 0, ((1, 0), (3, 1)) * 2, 16), None)
        b, h0 = g >> 2, 16 * ((g >> 1) & 1) + (g & 1)

        def score(i, s):
            q = qa_s[h0 + 2 * i, _blk(b, 8), :].astype(BF16)
            return jnp.where(_iota((8, WIN), 0) == i, _dot_nt(q, k_s[g, i]), s)
        s = _loop(8, score, jnp.zeros((8, WIN), F32), unroll=4) * SCALE
        p = jnp.exp(s - jnp.max(s, axis=1, keepdims=True))
        p16 = p.astype(BF16)

        def mix(i, o):
            return jnp.where(_iota((8, 128), 0) == i, _dot(p16, v_s[g, i]), o)
        o = _loop(8, mix, jnp.zeros((8, 128), F32), unroll=4) / jnp.sum(p, axis=1, keepdims=True)
        for i in range(8):
            oa_s[h0 + 2 * i] = jnp.where(_iota((8, 128), 0) == b, o[i:i + 1], oa_s[h0 + 2 * i])
    _loop(16, window_step)

    for i, (first, segments, rows) in enumerate(WO_TAIL):
        issue_wo(3, wo_sem.at[3 + i], first, segments, rows)
    acc = _loop(3, lambda j, acc: acc + project_a(0, 8, j, wo_sem.at[j]), jnp.zeros((8, 512), F32))
    for i, (first, segments, _) in enumerate(WO_TAIL):
        acc = acc + project_a(first, sum(n for n, _ in segments), 3, wo_sem.at[3 + i])
    out_s[:, :512] = acc[:4].astype(BF16)
    out_copy = pltpu.make_async_copy(out_s, out_h, x_sem.at[2])
    out_copy.start()
    out_copy.wait()


@jax.jit
def pallas_concat_heads__sliding_block_cached__compressed_kv_cla__decode_kernel(
    A_x: jax.Array,
    A_k_cache: jax.Array,
    A_v_cache: jax.Array,
    A_wq: jax.Array,
    A_wo: jax.Array,
    B_x: jax.Array,
    B_c_kv: jax.Array,
    B_w_q: jax.Array,
    B_w_uk: jax.Array,
    B_w_uv: jax.Array,
    B_w_o: jax.Array,
):
    operands = (
        A_x.reshape(4, 512),
        A_k_cache.reshape(8, 8, 2, SK, 128),
        A_v_cache.reshape(8, 8, 2, SK, 128),
        A_wq.reshape(4, 128, 4096),
        A_wo.reshape(8, 512, 512),
        B_x.reshape(4, 512),
        B_c_kv.reshape(8, 2, 1024, 512),
        B_w_q.reshape(4, 128, 32, 128),
        B_w_uk.reshape(4, 128, 32, 128),
        B_w_uv.reshape(4, 128, 32, 128),
        B_w_o.reshape(4, 1024, 512),
    )
    landing = [x.shape for x in operands]
    landing[1] = landing[2] = (16, 8, WIN, 128)
    vmem, dma = pltpu.VMEM, pltpu.SemaphoreType.DMA
    out = pl.pallas_call(
        _kernel,
        out_shape=jax.ShapeDtypeStruct((4, 1024), BF16),
        in_specs=[pl.BlockSpec(memory_space=pltpu.HBM)] * len(operands),
        out_specs=pl.BlockSpec(memory_space=pltpu.HBM),
        scratch_shapes=[
            *(vmem(shape, BF16) for shape in landing),
            vmem((2, 128, 1024), BF16),
            vmem((32, 512), BF16),
            vmem((4, 64, 128), BF16),
            vmem((2, 64, 128), BF16),
            vmem((4, 4, 32, 128), BF16),
            vmem((8, 32, 512), F32),
            vmem((4, 2, 64, 128), BF16),
            vmem((32, 32, 128), F32),
            vmem((32, 8, 128), F32),
            vmem((32, 8, 128), F32),
            vmem((4, 1024), BF16),
            dma((6,)), dma((16,)), dma((16,)), dma((3 + len(WO_TAIL),)), dma((3,)),
        ],
        compiler_params=pltpu.CompilerParams(
            vmem_limit_bytes=120 * 1024 * 1024,
            disable_bounds_checks=True,
            disable_semaphore_checks=True,
        ),
    )(*operands)
    return out.reshape(4, 1, 1024)
```
